```python
import jax
import jax.numpy as jnp

def _softmax(x, axis=-1):
    return jax.nn.softmax(x, axis=axis)
def _gelu(x):
    return jax.nn.gelu(x, approximate=True)
def _silu(x):
    return jax.nn.silu(x)
def _sigmoid(x):
    return jax.nn.sigmoid(x)
def _layernorm(x, axis=-1, eps=1e-5):
    m = jnp.mean(x, axis=axis, keepdims=True)
    v = jnp.var(x, axis=axis, keepdims=True)
    return (x - m) / jnp.sqrt(v + eps)
def _scatter_add(tgt, idx, src, axis=0):
    return tgt.at[idx].add(src)
def _segment_sum(src, seg, n):
    return jax.ops.segment_sum(src, seg, n)
class _Rng:
    def __init__(self, key):
        self._k = key
    def _next(self):
        self._k, sub = jax.random.split(self._k)
        return sub
    def normal(self, shape):
        return jax.random.normal(self._next(), shape, dtype=jnp.bfloat16)
    def randint(self, lo, hi, shape):
        return jax.random.randint(self._next(), shape, lo, hi, dtype=jnp.int32)
    def uniform(self, shape, lo=0.0, hi=1.0):
        return jax.random.uniform(self._next(), shape, jnp.bfloat16, lo, hi)
    def permutation(self, n):
        return jax.random.permutation(self._next(), n)


kernel_name = 'recurrent_scan__sliding_block_cached__mixer_s_mlp__decode'

def setup_inputs():
    _rng = _Rng(jax.random.key(int.from_bytes(__import__("os").urandom(4), "little")))
    _w = (lambda a: (lambda t: t.astype(jnp.bfloat16) if jnp.issubdtype(t.dtype, jnp.floating) else t)(jnp.asarray(a)))
    def _A_setup():
        B, Sq, D = 1, 1, 512
        Hq, Hkv, Sk, Dh = 32, 32, 32768, 128
        assert Hq % Hkv == 0, (Hq, Hkv)
        return {
            "x": _w((lambda *s: _rng.normal(s) * 0.05)(B, Sq, D)),
            "k_cache": _w((lambda *s: _rng.normal(s) * 0.05)(B, Hkv, Sk, Dh)),
            "v_cache": _w((lambda *s: _rng.normal(s) * 0.05)(B, Hkv, Sk, Dh)),
            "wq": _w((lambda *s: _rng.normal(s) * 0.05)(D, Hq * Dh) * (D ** -0.5)),
            "wo": _w((lambda *s: _rng.normal(s) * 0.05)(Hq * Dh, D) * ((Hq * Dh) ** -0.5)),
        }
    _A_in = _A_setup()

    def _B_setup():
        B, S, D, F = 1, 1, 512, 1376
        return {
            "x":  _w((lambda *s: _rng.normal(s) * 0.05)(B, S, D)),
            "w1": _w((lambda *s: _rng.normal(s) * 0.05)(D, D) * (D ** -0.5)),
            "w2": _w((lambda *s: _rng.normal(s) * 0.05)(D, D) * (D ** -0.5)),
            "w3": _w((lambda *s: _rng.normal(s) * 0.05)(D, F) * (D ** -0.5)),
            "w4": _w((lambda *s: _rng.normal(s) * 0.05)(F, D) * (F ** -0.5)),
        }
    _B_in = _B_setup()

    return {
        "A_x": _A_in["x"],
        "A_k_cache": _A_in["k_cache"],
        "A_v_cache": _A_in["v_cache"],
        "A_wq": _A_in["wq"],
        "A_wo": _A_in["wo"],
        "B_x": _B_in["x"],
        "B_w1": _B_in["w1"],
        "B_w2": _B_in["w2"],
        "B_w3": _B_in["w3"],
        "B_w4": _B_in["w4"],
    }

def reference(A_x, A_k_cache, A_v_cache, A_wq, A_wo, B_x, B_w1, B_w2, B_w3, B_w4):
    def _A_ref(x, k_cache, v_cache, wq, wo):
        B, Sq, D = x.shape
        Hq, Dh = 32, 128
        Hkv, Sk = k_cache.shape[1], k_cache.shape[2]
        W = min(4096, max(256, Sk // 4))
        rep = Hq // Hkv
        q = (lambda x, *d: x.transpose(*d))((x @ wq).reshape(B, Sq, Hq, Dh), 0, 2, 1, 3)
        k = jnp.repeat(k_cache[:, :, Sk - W:, :], rep, axis=1)
        v = jnp.repeat(v_cache[:, :, Sk - W:, :], rep, axis=1)
        scores = jnp.einsum("bhqd,bhkd->bhqk", q, k) * (Dh ** -0.5)
        p = _softmax(scores, axis=-1)
        o = jnp.einsum("bhqk,bhkd->bhqd", p, v)
        return (lambda x, *d: x.transpose(*d))(o, 0, 2, 1, 3).reshape(B, Sq, Hq * Dh) @ wo

    def _B_ref(x, w1, w2, w3, w4):
        B, S, D = x.shape
        h = _gelu(_layernorm(x, axis=-1) @ w1)
        c = D // 4
        g0 = jnp.pad(h[:, :, 0*c:1*c], ((0, 0), (1, 0), (0, 0)))[:, :S, :]
        g1 = jnp.pad(h[:, :, 1*c:2*c], ((0, 0), (0, 1), (0, 0)))[:, 1:, :]
        g2 = jnp.pad(h[:, :, 2*c:3*c], ((0, 0), (2, 0), (0, 0)))[:, :S, :]
        g3 = jnp.pad(h[:, :, 3*c:   ], ((0, 0), (0, 2), (0, 0)))[:, 2:, :]
        hs = jnp.concatenate([g0, g1, g2, g3], axis=-1) @ w2
        x1 = x + hs
        h2 = _gelu(_layernorm(x1, axis=-1) @ w3) @ w4
        return x1 + h2

    x = A_x
    xn = _layernorm(x, axis=-1)
    s = _A_ref(xn, A_k_cache, A_v_cache, A_wq, A_wo)
    g = _silu(_B_ref(xn, B_w1, B_w2, B_w3, B_w4))
    return x + s * g
```

```python
import functools

import jax
import jax.numpy as jnp
import jax.experimental.pallas as pl
import jax.experimental.pallas.tpu as pltpu

_NT = (((1,), (1,)), ((), ()))
_ROWS = 8


def _layernorm(x, eps=1e-5):
    m = jnp.mean(x, axis=-1, keepdims=True)
    d = x - m
    v = jnp.mean(d * d, axis=-1, keepdims=True)
    return d / jnp.sqrt(v + eps)


def _sigmoid(x):
    return 1.0 / (1.0 + jnp.exp(-x))


def _starts(sizes):
    out, s = [], 0
    for c in sizes:
        out.append(s)
        s += c
    return out


def _kernel(x_hbm, k_hbm, v_hbm, wq_hbm, wo_hbm, w3t_hbm, w4_hbm, o_ref,
            x_v, k_v, v_v, wq_v, wo_v, w3t_v, w4_v, q_s, o_s,
            w_sem, k_sem, v_sem, wo_sem, *, w0, kv_chunks, wo_chunks, depth, prio):
    f32, bf16 = jnp.float32, jnp.bfloat16
    H, W, Dh = k_v.shape
    D = x_v.shape[-1]

    def cache_copy(src, dst, sem, i, s, c):
        return pltpu.make_async_copy(
            src.at[0, pl.ds(s, c), pl.ds(w0, W), :], dst.at[pl.ds(s, c)], sem.at[i])

    kv = list(zip(_starts(kv_chunks), kv_chunks))
    k_cp = [cache_copy(k_hbm, k_v, k_sem, i, s, c) for i, (s, c) in enumerate(kv)]
    v_cp = [cache_copy(v_hbm, v_v, v_sem, i, s, c) for i, (s, c) in enumerate(kv)]
    woc = list(zip(_starts(wo_chunks), wo_chunks))
    wo_cp = [
        pltpu.make_async_copy(wo_hbm.at[pl.ds(s * Dh, c * Dh)],
                              wo_v.at[pl.ds(s * Dh, c * Dh)], wo_sem.at[i])
        for i, (s, c) in enumerate(woc)
    ]
    wq_cp = pltpu.make_async_copy(wq_hbm, wq_v, w_sem.at[0])
    x_cp = pltpu.make_async_copy(x_hbm, x_v, w_sem.at[1])
    w3_cp = pltpu.make_async_copy(w3t_hbm, w3t_v, w_sem.at[2])
    w4_cp = pltpu.make_async_copy(w4_hbm, w4_v, w_sem.at[3])

    stream = [wq_cp]
    for kc, vc in zip(k_cp, v_cp):
        stream += [kc, vc]
    stream += [w3_cp, w4_cp] + wo_cp

    def land(cp):
        cp.wait()
        nxt = next(i for i, c in enumerate(stream) if c is cp) + depth
        if nxt < len(stream):
            stream[nxt].start(priority=nxt % prio)

    for i, cp in enumerate(stream[:depth]):
        cp.start(priority=i % prio)
    x_cp.start()

    x_cp.wait()
    x = jnp.broadcast_to(x_v[0].astype(f32), (_ROWS, D))
    xn = _layernorm(x).astype(bf16)

    land(wq_cp)

    def q_body(h, _):
        col = pl.multiple_of(h * Dh, Dh)
        q_s[h] = jnp.dot(xn, wq_v[:, pl.ds(col, Dh)], preferred_element_type=f32)
        return _

    jax.lax.fori_loop(0, H, q_body, 0, unroll=4)

    def head_body(h, _):
        for (s, c), kc in zip(kv, k_cp):
            pl.when(h == s)(functools.partial(land, kc))
        sc = jax.lax.dot_general(q_s[h].astype(bf16), k_v[h], _NT,
                                 preferred_element_type=f32) * (Dh ** -0.5)
        p = jnp.exp(sc - jnp.max(sc, axis=-1, keepdims=True))
        l = jnp.sum(p, axis=-1, keepdims=True)
        for (s, c), vc in zip(kv, v_cp):
            pl.when(h == s)(functools.partial(land, vc))
        o = jnp.dot(p.astype(bf16), v_v[h], preferred_element_type=f32)
        o_s[:, pl.ds(pl.multiple_of(h * Dh, Dh), Dh)] = o / l
        return _

    jax.lax.fori_loop(0, H, head_body, 0)

    x1 = xn.astype(f32)
    land(w3_cp)
    hid = jax.lax.dot_general(_layernorm(x1).astype(bf16), w3t_v[...], _NT,
                              preferred_element_type=f32)
    hid = jax.nn.gelu(hid, approximate=True).astype(bf16)
    land(w4_cp)
    b = x1 + jnp.dot(hid, w4_v[...], preferred_element_type=f32)
    g = b * _sigmoid(b)

    acc = jnp.zeros((_ROWS, D), f32)
    for (s, c), cp in zip(woc, wo_cp):
        rows = slice(s * Dh, (s + c) * Dh)
        o = o_s[:, rows].astype(bf16)
        land(cp)
        acc = acc + jnp.dot(o, wo_v[rows, :], preferred_element_type=f32)

    o_ref[0] = (x + acc * g)[:1].astype(o_ref.dtype)


def _build(A_x, A_k_cache, A_v_cache, A_wq, A_wo, B_w3, B_w4,
           kv_chunks=(8, 8, 8, 4, 4), wo_chunks=(12, 8, 6, 4, 2), depth=3, prio=2):
    B, S, D = A_x.shape
    _, H, Sk, Dh = A_k_cache.shape
    F = B_w3.shape[1]
    W = min(4096, max(256, Sk // 4))
    assert B == 1 and S == 1 and A_wq.shape[1] == H * Dh
    assert sum(kv_chunks) == H and sum(wo_chunks) == H
    dt = A_x.dtype
    dma = pltpu.SemaphoreType.DMA
    return pl.pallas_call(
        functools.partial(_kernel, w0=Sk - W, kv_chunks=kv_chunks, wo_chunks=wo_chunks,
                          depth=depth, prio=prio),
        in_specs=[pl.BlockSpec(memory_space=pl.ANY)] * 7,
        out_shape=jax.ShapeDtypeStruct((B, S, D), dt),
        scratch_shapes=[
            pltpu.VMEM((B, S, D), dt),
            pltpu.VMEM((H, W, Dh), dt),
            pltpu.VMEM((H, W, Dh), dt),
            pltpu.VMEM((D, H * Dh), dt),
            pltpu.VMEM((H * Dh, D), dt),
            pltpu.VMEM((F, D), dt),
            pltpu.VMEM((F, D), dt),
            pltpu.VMEM((H, _ROWS, Dh), jnp.float32),
            pltpu.VMEM((_ROWS, H * Dh), jnp.float32),
            dma((4,)), dma((len(kv_chunks),)), dma((len(kv_chunks),)), dma((len(wo_chunks),)),
        ],
        compiler_params=pltpu.CompilerParams(vmem_limit_bytes=100 * 2**20),
    )(A_x, A_k_cache, A_v_cache, A_wq, A_wo, B_w3.T, B_w4)


@jax.jit
def pallas_recurrent_scan__sliding_block_cached__mixer_s_mlp__decode_kernel(
    A_x: jax.Array,
    A_k_cache: jax.Array,
    A_v_cache: jax.Array,
    A_wq: jax.Array,
    A_wo: jax.Array,
    B_x: jax.Array,
    B_w1: jax.Array,
    B_w2: jax.Array,
    B_w3: jax.Array,
    B_w4: jax.Array,
):
    return _build(A_x, A_k_cache, A_v_cache, A_wq, A_wo, B_w3, B_w4)
```
